```python
import os as _os
_os.environ.setdefault("JAX_PLATFORMS", "cpu")
import jax
import jax.numpy as jnp

def _softmax(x, axis=-1):
    return jax.nn.softmax(x, axis=axis)
def _gelu(x):
    return jax.nn.gelu(x, approximate=True)
def _silu(x):
    return jax.nn.silu(x)
def _sigmoid(x):
    return jax.nn.sigmoid(x)
def _layernorm(x, axis=-1, eps=1e-5):
    m = jnp.mean(x, axis=axis, keepdims=True)
    v = jnp.var(x, axis=axis, keepdims=True)
    return (x - m) / jnp.sqrt(v + eps)
def _scatter_add(tgt, idx, src, axis=0):
    return tgt.at[idx].add(src)
def _segment_sum(src, seg, n):
    return jax.ops.segment_sum(src, seg, n)
class _Rng:
    def __init__(self, key):
        self._k = key
    def _next(self):
        self._k, sub = jax.random.split(self._k)
        return sub
    def normal(self, shape):
        return jax.random.normal(self._next(), shape, dtype=jnp.bfloat16)
    def randint(self, lo, hi, shape):
        return jax.random.randint(self._next(), shape, lo, hi, dtype=jnp.int32)
    def uniform(self, shape, lo=0.0, hi=1.0):
        return jax.random.uniform(self._next(), shape, jnp.bfloat16, lo, hi)
    def permutation(self, n):
        return jax.random.permutation(self._next(), n)


kernel_name = 'standalone__dense_activation_gelu__prompt'

def setup_inputs():
    _rng = _Rng(jax.random.key(int.from_bytes(__import__("os").urandom(4), "little")))
    _w = (lambda a: (lambda t: t.astype(jnp.bfloat16) if jnp.issubdtype(t.dtype, jnp.floating) else t)(jnp.asarray(a)))
    B, S, D, F = 1, 2048, 640, 1728
    return {
        "x": _w((lambda *s: _rng.normal(s) * 0.05)(B, S, D)),
        "w1": _w((lambda *s: _rng.normal(s) * 0.05)(D, F) * (D ** -0.5)),
        "b1": _w((lambda *s: _rng.normal(s) * 0.05)(F) * 0.01),
        "w2": _w((lambda *s: _rng.normal(s) * 0.05)(F, D) * (F ** -0.5)),
        "b2": _w((lambda *s: _rng.normal(s) * 0.05)(D) * 0.01),
    }

def reference(x, w1, b1, w2, b2):
    h = jnp.einsum("bsd,df->bsf", x, w1) + b1
    h = _gelu(h)
    return jnp.einsum("bsf,fd->bsd", h, w2) + b2
```

```python
import jax
import jax.numpy as jnp
from jax import lax
import jax.experimental.pallas as pl
import jax.experimental.pallas.tpu as pltpu

TM = 512
TS = 256
WP = 128
FIRST_CHUNKS = (128, 256, 640, 704)
VMEM_LIMIT_BYTES = 64 * 1024 * 1024

_NT = (((1,), (1,)), ((), ()))


def _act(h, b1):
    return jax.nn.gelu(h + b1, approximate=True).astype(jnp.bfloat16)


def _mlp_kernel(b1_hbm, b2_hbm, x_hbm, w1t_hbm, w2_hbm, o_hbm,
                x_v, o_v, w1t_v, w2_v, b1_v, b2_v,
                w1sem, w2sem, xsem, osem, bsem):
    pid = pl.program_id(0)
    last = pl.num_programs(0) - 1
    F = w1t_v.shape[0]
    S = x_v.shape[0]
    nx = S // TS
    nsub = TM // TS
    chunks = FIRST_CHUNKS
    starts = [sum(chunks[:k]) for k in range(len(chunks))]
    n_full = F // WP
    rem = F - n_full * WP

    def w_piece(i, r0, rows):
        return (
            pltpu.make_async_copy(w1t_hbm.at[pl.ds(r0, rows), :], w1t_v.at[pl.ds(r0, rows), :], w1sem.at[i]),
            pltpu.make_async_copy(w2_hbm.at[pl.ds(r0, rows), :], w2_v.at[pl.ds(r0, rows), :], w2sem.at[i]),
        )

    def x_copy(i):
        return pltpu.make_async_copy(x_hbm.at[0, pl.ds(i * TS, TS), :], x_v.at[pl.ds(i * TS, TS), :], xsem.at[i])

    def o_copy(i, r0):
        return pltpu.make_async_copy(o_v.at[pl.ds(r0, TS), :], o_hbm.at[0, pl.ds(r0, TS), :], osem.at[i])

    def b_copies():
        return (pltpu.make_async_copy(b1_hbm, b1_v, bsem.at[0]),
                pltpu.make_async_copy(b2_hbm, b2_v, bsem.at[1]))

    @pl.when(pid == 0)
    def _first():
        for c in b_copies():
            c.start()
        for i in range(nsub):
            x_copy(i).start()

        def issue_w(i, carry):
            a, b = w_piece(i, pl.multiple_of(i * WP, WP), WP)
            a.start()
            b.start()
            return carry
        lax.fori_loop(0, n_full, issue_w, 0)
        if rem:
            a, b = w_piece(n_full, n_full * WP, rem)
            a.start()
            b.start()

        def issue_x(i, carry):
            r0 = pl.multiple_of(i * TS, TS)
            pltpu.make_async_copy(x_hbm.at[0, pl.ds(r0, TS), :], x_v.at[pl.ds(r0, TS), :], xsem.at[i]).start()
            return carry
        lax.fori_loop(nsub, nx, issue_x, 0)

        for c in b_copies():
            c.wait()
        for i in range(nsub):
            x_copy(i).wait()
        b2 = b2_v[...].astype(jnp.float32)[None, :]
        accs = [None] * nsub
        for k in range(len(chunks)):
            c0, n = starts[k], chunks[k]
            for i in range(c0 // WP, -(-(c0 + n) // WP)):
                a, b = w_piece(i, i * WP, min(WP, F - i * WP))
                a.wait()
                b.wait()
            b1k = b1_v[c0:c0 + n].astype(jnp.float32)[None, :]
            for s in range(nsub):
                h = lax.dot_general(x_v[s * TS:(s + 1) * TS, :], w1t_v[c0:c0 + n, :], _NT,
                                    preferred_element_type=jnp.float32)
                p = jnp.dot(_act(h, b1k), w2_v[c0:c0 + n, :], preferred_element_type=jnp.float32)
                accs[s] = p if k == 0 else accs[s] + p
                if k == len(chunks) - 1:
                    o_v[s * TS:(s + 1) * TS, :] = (accs[s] + b2).astype(o_v.dtype)
                    o_copy(s, s * TS).start()
        for i in range(nsub, nx):
            x_copy(i).wait()

    @pl.when(pid > 0)
    def _steady():
        b1 = b1_v[...].astype(jnp.float32)[None, :]
        b2 = b2_v[...].astype(jnp.float32)[None, :]
        for s in range(nsub):
            r0 = pl.multiple_of(pid * TM + s * TS, TS)
            h = lax.dot_general(x_v[pl.ds(r0, TS), :], w1t_v[...], _NT, preferred_element_type=jnp.float32)
            y = jnp.dot(_act(h, b1), w2_v[...], preferred_element_type=jnp.float32) + b2
            o_v[pl.ds(r0, TS), :] = y.astype(o_v.dtype)
            o_copy(pid * nsub + s, r0).start()

    @pl.when(pid == last)
    def _drain():
        for i in range(nx):
            o_copy(i, i * TS).wait()


@jax.jit
def pallas_standalone__dense_activation_gelu__prompt_kernel(
    x: jax.Array,
    w1: jax.Array,
    b1: jax.Array,
    w2: jax.Array,
    b2: jax.Array,
):
    B, S, D = x.shape
    F = w1.shape[1]
    assert B == 1 and S % TM == 0 and TM % TS == 0
    assert sum(FIRST_CHUNKS) == F and w2.shape == (F, D)
    n_pieces = pl.cdiv(F, WP)
    return pl.pallas_call(
        _mlp_kernel,
        grid=(S // TM,),
        in_specs=[pl.BlockSpec(memory_space=pl.ANY)] * 5,
        out_specs=pl.BlockSpec(memory_space=pl.ANY),
        out_shape=jax.ShapeDtypeStruct((B, S, D), x.dtype),
        scratch_shapes=[
            pltpu.VMEM((S, D), x.dtype),
            pltpu.VMEM((S, D), x.dtype),
            pltpu.VMEM((F, D), w1.dtype),
            pltpu.VMEM((F, D), w2.dtype),
            pltpu.VMEM((F,), b1.dtype),
            pltpu.VMEM((D,), b2.dtype),
            pltpu.SemaphoreType.DMA((n_pieces,)),
            pltpu.SemaphoreType.DMA((n_pieces,)),
            pltpu.SemaphoreType.DMA((S // TS,)),
            pltpu.SemaphoreType.DMA((S // TS,)),
            pltpu.SemaphoreType.DMA((2,)),
        ],
        compiler_params=pltpu.CompilerParams(
            dimension_semantics=("arbitrary",),
            vmem_limit_bytes=VMEM_LIMIT_BYTES,
        ),
    )(b1, b2, x, w1.T, w2)
```

```python
import jax
import jax.numpy as jnp
from jax import lax
import jax.experimental.pallas as pl
import jax.experimental.pallas.tpu as pltpu

TM = 512
TS = 256
WP = 128
FIRST_CHUNKS = (128, 256, 640, 704)
OUT_BLOCKS = (512, 128)
VMEM_LIMIT_BYTES = 64 * 1024 * 1024

_NT = (((1,), (1,)), ((), ()))


def _act(h, b1):
    return jax.nn.gelu(h + b1, approximate=True).astype(jnp.bfloat16)


def _mlp_kernel(b1_hbm, b2_hbm, x_hbm, w1t_hbm, w2_hbm, o_hbm,
                x_v, o_v, w1t_v, w2_v, b1_v, b2_v,
                w1sem, w2sem, xsem, osem, bsem):
    pid = pl.program_id(0)
    last = pl.num_programs(0) - 1
    F = w1t_v.shape[0]
    S = x_v.shape[0]
    nx = S // TS
    nsub = TM // TS
    chunks = FIRST_CHUNKS
    starts = [sum(chunks[:k]) for k in range(len(chunks))]
    n_full = F // WP
    rem = F - n_full * WP

    def w_piece(i, r0, rows):
        return (
            pltpu.make_async_copy(w1t_hbm.at[pl.ds(r0, rows), :], w1t_v.at[pl.ds(r0, rows), :], w1sem.at[i]),
            pltpu.make_async_copy(w2_hbm.at[pl.ds(r0, rows), :], w2_v.at[pl.ds(r0, rows), :], w2sem.at[i]),
        )

    def x_copy(i):
        return pltpu.make_async_copy(x_hbm.at[0, pl.ds(i * TS, TS), :], x_v.at[pl.ds(i * TS, TS), :], xsem.at[i])

    ob = OUT_BLOCKS
    ostarts = [sum(ob[:j]) for j in range(len(ob))]

    def o_copy(i, r0, j):
        return pltpu.make_async_copy(o_v.at[pl.ds(r0, TS), pl.ds(ostarts[j], ob[j])],
                                     o_hbm.at[0, pl.ds(r0, TS), pl.ds(ostarts[j], ob[j])],
                                     osem.at[i * len(ob) + j])

    def store_out(i, r0, y):
        yb = y.astype(o_v.dtype)
        for j in range(len(ob)):
            o_v[pl.ds(r0, TS), ostarts[j]:ostarts[j] + ob[j]] = yb[:, ostarts[j]:ostarts[j] + ob[j]]
            o_copy(i, r0, j).start()

    def mlp(xs, b1, c0, n):
        nm = (n // 128) * 128
        h = lax.dot_general(xs, w1t_v[c0:c0 + nm, :], _NT, preferred_element_type=jnp.float32)
        if nm < n:
            ht = lax.dot_general(w1t_v[c0 + nm:c0 + n, :], xs, _NT, preferred_element_type=jnp.float32)
            gr = _act(ht.T, b1[:, c0 + nm:c0 + n])
        y = jnp.dot(_act(h, b1[:, c0:c0 + nm]), w2_v[c0:c0 + nm, :], preferred_element_type=jnp.float32)
        if nm < n:
            y = y + jnp.dot(gr, w2_v[c0 + nm:c0 + n, :], preferred_element_type=jnp.float32)
        return y

    def b_copies():
        return (pltpu.make_async_copy(b1_hbm, b1_v, bsem.at[0]),
                pltpu.make_async_copy(b2_hbm, b2_v, bsem.at[1]))

    @pl.when(pid == 0)
    def _first():
        for c in b_copies():
            c.start()
        for i in range(nsub):
            x_copy(i).start()

        def issue_w(i, carry):
            a, b = w_piece(i, pl.multiple_of(i * WP, WP), WP)
            a.start()
            b.start()
            return carry
        lax.fori_loop(0, n_full, issue_w, 0)
        if rem:
            a, b = w_piece(n_full, n_full * WP, rem)
            a.start()
            b.start()

        def issue_x(i, carry):
            r0 = pl.multiple_of(i * TS, TS)
            pltpu.make_async_copy(x_hbm.at[0, pl.ds(r0, TS), :], x_v.at[pl.ds(r0, TS), :], xsem.at[i]).start()
            return carry
        lax.fori_loop(nsub, nx, issue_x, 0)

        for c in b_copies():
            c.wait()
        for i in range(nsub):
            x_copy(i).wait()
        b1 = b1_v[...].astype(jnp.float32)[None, :]
        b2 = b2_v[...].astype(jnp.float32)[None, :]
        accs = [None] * nsub
        for k in range(len(chunks)):
            c0, n = starts[k], chunks[k]
            for i in range(c0 // WP, -(-(c0 + n) // WP)):
                a, b = w_piece(i, i * WP, min(WP, F - i * WP))
                a.wait()
                b.wait()
            for s in range(nsub):
                p = mlp(x_v[s * TS:(s + 1) * TS, :], b1, c0, n)
                accs[s] = p if k == 0 else accs[s] + p
                if k == len(chunks) - 1:
                    store_out(s, s * TS, accs[s] + b2)
        for i in range(nsub, nx):
            x_copy(i).wait()

    @pl.when(pid > 0)
    def _steady():
        b1 = b1_v[...].astype(jnp.float32)[None, :]
        b2 = b2_v[...].astype(jnp.float32)[None, :]
        for s in range(nsub):
            r0 = pl.multiple_of(pid * TM + s * TS, TS)
            y = mlp(x_v[pl.ds(r0, TS), :], b1, 0, F) + b2
            store_out(pid * nsub + s, r0, y)

    @pl.when(pid == last)
    def _drain():
        for i in range(nx):
            for j in range(len(ob)):
                o_copy(i, i * TS, j).wait()


@jax.jit
def pallas_standalone__dense_activation_gelu__prompt_kernel(
    x: jax.Array,
    w1: jax.Array,
    b1: jax.Array,
    w2: jax.Array,
    b2: jax.Array,
):
    B, S, D = x.shape
    F = w1.shape[1]
    assert B == 1 and S % TM == 0 and TM % TS == 0
    assert sum(FIRST_CHUNKS) == F and w2.shape == (F, D) and sum(OUT_BLOCKS) == D
    assert all(sum(FIRST_CHUNKS[:k]) % WP == 0 for k in range(len(FIRST_CHUNKS)))
    n_pieces = pl.cdiv(F, WP)
    return pl.pallas_call(
        _mlp_kernel,
        grid=(S // TM,),
        in_specs=[pl.BlockSpec(memory_space=pl.ANY)] * 5,
        out_specs=pl.BlockSpec(memory_space=pl.ANY),
        out_shape=jax.ShapeDtypeStruct((B, S, D), x.dtype),
        scratch_shapes=[
            pltpu.VMEM((S, D), x.dtype),
            pltpu.VMEM((S, D), x.dtype),
            pltpu.VMEM((F, D), w1.dtype),
            pltpu.VMEM((F, D), w2.dtype),
            pltpu.VMEM((F,), b1.dtype),
            pltpu.VMEM((D,), b2.dtype),
            pltpu.SemaphoreType.DMA((n_pieces,)),
            pltpu.SemaphoreType.DMA((n_pieces,)),
            pltpu.SemaphoreType.DMA((S // TS,)),
            pltpu.SemaphoreType.DMA((S // TS * len(OUT_BLOCKS),)),
            pltpu.SemaphoreType.DMA((2,)),
        ],
        compiler_params=pltpu.CompilerParams(
            dimension_semantics=("arbitrary",),
            vmem_limit_bytes=VMEM_LIMIT_BYTES,
        ),
    )(b1, b2, x, w1.T, w2)
```
